```python
import os as _os
_os.environ.setdefault("JAX_PLATFORMS", "cpu")
import jax
import jax.numpy as jnp

def _softmax(x, axis=-1):
    return jax.nn.softmax(x, axis=axis)
def _gelu(x):
    return jax.nn.gelu(x, approximate=True)
def _silu(x):
    return jax.nn.silu(x)
def _sigmoid(x):
    return jax.nn.sigmoid(x)
def _layernorm(x, axis=-1, eps=1e-5):
    m = jnp.mean(x, axis=axis, keepdims=True)
    v = jnp.var(x, axis=axis, keepdims=True)
    return (x - m) / jnp.sqrt(v + eps)
def _scatter_add(tgt, idx, src, axis=0):
    return tgt.at[idx].add(src)
def _segment_sum(src, seg, n):
    return jax.ops.segment_sum(src, seg, n)
class _Rng:
    def __init__(self, key):
        self._k = key
    def _next(self):
        self._k, sub = jax.random.split(self._k)
        return sub
    def normal(self, shape):
        return jax.random.normal(self._next(), shape, dtype=jnp.bfloat16)
    def randint(self, lo, hi, shape):
        return jax.random.randint(self._next(), shape, lo, hi, dtype=jnp.int32)
    def uniform(self, shape, lo=0.0, hi=1.0):
        return jax.random.uniform(self._next(), shape, jnp.bfloat16, lo, hi)
    def permutation(self, n):
        return jax.random.permutation(self._next(), n)


kernel_name = 'standalone__gqa_block_cached__near_ridge'

def setup_inputs():
    _rng = _Rng(jax.random.key(int.from_bytes(__import__("os").urandom(4), "little")))
    _w = (lambda a: (lambda t: t.astype(jnp.bfloat16) if jnp.issubdtype(t.dtype, jnp.floating) else t)(jnp.asarray(a)))
    B, Sq, D = 8, 96, 448
    Hq, Hkv, Sk, Dh = 16, 8, 2048, 256
    assert Hq % Hkv == 0, (Hq, Hkv)
    return {
        "x": _w((lambda *s: _rng.normal(s) * 0.8)(B, Sq, D)),
        "k_cache": _w((lambda *s: _rng.normal(s) * 0.8)(B, Hkv, Sk, Dh)),
        "v_cache": _w((lambda *s: _rng.normal(s) * 0.05)(B, Hkv, Sk, Dh)),
        "wq": _w((lambda *s: _rng.normal(s) * 0.8)(D, Hq * Dh) * (D ** -0.5)),
        "wo": _w((lambda *s: _rng.normal(s) * 0.05)(Hq * Dh, D) * ((Hq * Dh) ** -0.5)),
    }

def reference(x, k_cache, v_cache, wq, wo):
    B, Sq, D = x.shape
    Hq, Dh = 16, 256
    Hkv = k_cache.shape[1]
    rep = Hq // Hkv
    q = (lambda x, *d: x.transpose(*d))((x @ wq).reshape(B, Sq, Hq, Dh), 0, 2, 1, 3)
    k = jnp.repeat(k_cache, rep, axis=1)
    v = jnp.repeat(v_cache, rep, axis=1)
    scores = jnp.einsum("bhqd,bhkd->bhqk", q, k) * (Dh ** -0.5)
    p = _softmax(scores, axis=-1)
    o = jnp.einsum("bhqk,bhkd->bhqd", p, v)
    return (lambda x, *d: x.transpose(*d))(o, 0, 2, 1, 3).reshape(B, Sq, Hq * Dh) @ wo
```

```python
import functools

import jax
import jax.numpy as jnp
from jax import lax
import jax.experimental.pallas as pl
import jax.experimental.pallas.tpu as pltpu

NB = 4
CH = 256
LAG = 2
OLAST = 1


def _kernel(x_hbm, k_hbm, v_hbm, wq_hbm, wot_hbm, out_hbm,
            x_v, wq_v, wo_v, kbuf, vbuf, s_buf, m_buf, acc, ostage,
            sem_x, sem_wq, sem_wo, sem_k, sem_v, sem_o,
            *, B, Hkv, rep, Sq, Sk, Dh, scale):
    T = B * Hkv
    W = rep * Dh
    NC = Sk // CH
    R = rep * Sq

    def k_copy(t):
        return pltpu.make_async_copy(k_hbm.at[t], kbuf.at[t % NB], sem_k.at[t % NB])

    def v_copy(t):
        return pltpu.make_async_copy(v_hbm.at[t], vbuf.at[t % NB], sem_v.at[t % NB])

    def wq_copy(h):
        return pltpu.make_async_copy(wq_hbm.at[:, pl.ds(h * W, W)], wq_v.at[h], sem_wq.at[h])

    def wo_copy(h):
        return pltpu.make_async_copy(wot_hbm.at[:, pl.ds(h * W, W)], wo_v.at[h], sem_wo.at[h])

    x_copy = pltpu.make_async_copy(x_hbm, x_v, sem_x.at[0])

    def o_copy(b):
        return pltpu.make_async_copy(ostage.at[b % 2], out_hbm.at[b], sem_o.at[b % 2])

    def fold(a, op):
        r = a[:, 0:128]
        for c in range(1, a.shape[1] // 128):
            r = op(r, a[:, c * 128:(c + 1) * 128])
        return r

    def qproj(t):
        b = t // Hkv
        h = t % Hkv
        x = x_v[b]
        qs = []
        for r in range(rep):
            q_r = jnp.dot(x, wq_v[h, :, r * Dh:(r + 1) * Dh], preferred_element_type=jnp.float32)
            qs.append((q_r.astype(jnp.bfloat16) * scale).astype(jnp.bfloat16))
        return jnp.concatenate(qs, axis=0)

    def qk(t, q, j, mx):
        s = lax.dot_general(q, kbuf[t % NB, j * CH:(j + 1) * CH, :], (((1,), (1,)), ((), ())),
                            preferred_element_type=jnp.float32)
        s_buf[:, j * CH:(j + 1) * CH] = s
        f = fold(s, jnp.maximum)
        return f if mx is None else jnp.maximum(mx, f)

    def a_fin(mx):
        m = jnp.max(mx, axis=-1, keepdims=True)
        m_buf[...] = jnp.broadcast_to(m, (R, 128))

    def expc(j, ls):
        m = m_buf[...]
        m2 = jnp.concatenate([m] * (CH // 128), axis=1)
        p = jnp.exp(s_buf[:, j * CH:(j + 1) * CH] - m2)
        f = fold(p, jnp.add)
        return p.astype(jnp.bfloat16), (f if ls is None else ls + f)

    def pv(t, j, p, o):
        d = jnp.dot(p, vbuf[t % NB, j * CH:(j + 1) * CH, :], preferred_element_type=jnp.float32)
        return d if o is None else o + d

    def b_fin(t, o, ls):
        h = t % Hkv
        l = jnp.sum(ls, axis=-1, keepdims=True)
        o = (o / l).astype(jnp.bfloat16)
        o_cat = jnp.concatenate([o[r * Sq:(r + 1) * Sq] for r in range(rep)], axis=1)
        contrib = lax.dot_general(o_cat, wo_v[h], (((1,), (1,)), ((), ())), preferred_element_type=jnp.float32)
        acc[...] += contrib

    def stage_a(t):
        q = qproj(t)
        mx = None
        for j in range(NC):
            mx = qk(t, q, j, mx)
        a_fin(mx)

    def stage_b(t):
        ls = None
        o = None
        p_next, ls = expc(0, ls)
        for j in range(NC):
            p = p_next
            if j + 1 < NC:
                p_next, ls = expc(j + 1, ls)
            o = pv(t, j, p, o)
        b_fin(t, o, ls)

    def stage_ab(tb):
        ta = tb + 1
        ls = None
        o = None
        mx = None
        p_next, ls = expc(0, ls)
        q = qproj(ta)
        nq = 0
        for j in range(NC):
            p = p_next
            if j + 1 < NC:
                p_next, ls = expc(j + 1, ls)
            o = pv(tb, j, p, o)
            if j >= LAG - 1 and nq < NC - LAG:
                mx = qk(ta, q, nq, mx)
                nq += 1
        if OLAST:
            while nq < NC:
                mx = qk(ta, q, nq, mx)
                nq += 1
            a_fin(mx)
            b_fin(tb, o, ls)
        else:
            while nq < NC - LAG + 1:
                mx = qk(ta, q, nq, mx)
                nq += 1
            b_fin(tb, o, ls)
            while nq < NC:
                mx = qk(ta, q, nq, mx)
                nq += 1
            a_fin(mx)

    def finish_batch(t):
        b = t // Hkv

        @pl.when(t % Hkv == Hkv - 1)
        def _():
            @pl.when(b >= 2)
            def _():
                o_copy(b - 2).wait()
            ostage[b % 2] = acc[...].astype(ostage.dtype)
            acc[...] = jnp.zeros_like(acc)
            o_copy(b).start()

    x_copy.start()
    wq_copy(0).start()
    k_copy(0).start()
    for t in range(1, Hkv + 1):
        if t < Hkv:
            wq_copy(t).start()
        if t < NB:
            k_copy(t).start()
        wo_copy(t - 1).start()
        if t < NB:
            v_copy(t - 1).start()
    acc[...] = jnp.zeros_like(acc)
    x_copy.wait()
    wq_copy(0).wait()
    k_copy(0).wait()
    stage_a(0)

    def body(i, carry):
        @pl.when(i + NB < T)
        def _():
            k_copy(i + NB).start()

        @pl.when(i + NB - 1 < T)
        def _():
            v_copy(i + NB - 1).start()

        @pl.when(i < Hkv)
        def _():
            wo_copy(i).wait()

            @pl.when(i < Hkv - 1)
            def _():
                wq_copy(i + 1).wait()
        k_copy(i + 1).wait()
        v_copy(i).wait()
        stage_ab(i)
        finish_batch(i)
        return carry

    lax.fori_loop(0, T - 1, body, 0)

    v_copy(T - 1).wait()
    stage_b(T - 1)
    finish_batch(T - 1)
    o_copy(B - 2).wait()
    o_copy(B - 1).wait()


@jax.jit
def pallas_standalone__gqa_block_cached__near_ridge_kernel(x, k_cache, v_cache, wq, wo):
    B, Sq, D = x.shape
    _, Hkv, Sk, Dh = k_cache.shape
    Hq = wq.shape[1] // Dh
    rep = Hq // Hkv
    scale = Dh ** -0.5
    W = rep * Dh
    k3 = k_cache.reshape(B * Hkv, Sk, Dh)
    v3 = v_cache.reshape(B * Hkv, Sk, Dh)
    wot = wo.T

    kernel = functools.partial(_kernel, B=B, Hkv=Hkv, rep=rep, Sq=Sq, Sk=Sk, Dh=Dh, scale=scale)
    any_spec = pl.BlockSpec(memory_space=pl.ANY)
    return pl.pallas_call(
        kernel,
        in_specs=[any_spec] * 5,
        out_specs=any_spec,
        out_shape=jax.ShapeDtypeStruct((B, Sq, D), x.dtype),
        scratch_shapes=[
            pltpu.VMEM((B, Sq, D), x.dtype),
            pltpu.VMEM((Hkv, D, W), wq.dtype),
            pltpu.VMEM((Hkv, D, W), wo.dtype),
            pltpu.VMEM((NB, Sk, Dh), k_cache.dtype),
            pltpu.VMEM((NB, Sk, Dh), v_cache.dtype),
            pltpu.VMEM((rep * Sq, Sk), jnp.float32),
            pltpu.VMEM((rep * Sq, 128), jnp.float32),
            pltpu.VMEM((Sq, D), jnp.float32),
            pltpu.VMEM((2, Sq, D), x.dtype),
            pltpu.SemaphoreType.DMA((1,)),
            pltpu.SemaphoreType.DMA((Hkv,)),
            pltpu.SemaphoreType.DMA((Hkv,)),
            pltpu.SemaphoreType.DMA((NB,)),
            pltpu.SemaphoreType.DMA((NB,)),
            pltpu.SemaphoreType.DMA((2,)),
        ],
        compiler_params=pltpu.CompilerParams(vmem_limit_bytes=64 * 1024 * 1024),
    )(x, k3, v3, wq, wot)
```

```python
import functools

import jax
import jax.numpy as jnp
from jax import lax
import jax.experimental.pallas as pl
import jax.experimental.pallas.tpu as pltpu

NB = 6
CH = 256
LAG = 2
NSPLIT = 20
LANES = 128


def _kernel(x_hbm, k_hbm, v_hbm, wq_hbm, wot_hbm, out_hbm,
            x_v, wq_v, wo_v, q_all, kbuf, vbuf, s_buf, m_buf, p_buf, l_buf, acc, ostage, sem,
            *, B, Hkv, rep, Sq, Sk, Dh, scale):
    T = B * Hkv
    W = rep * Dh
    NC = Sk // CH
    R = rep * Sq
    SEM_X = 0
    SEM_WQ = 1
    SEM_WO = SEM_WQ + Hkv
    SEM_K = SEM_WO + Hkv
    SEM_V = SEM_K + NB
    SEM_O = SEM_V + NB
    NT = (((1,), (1,)), ((), ()))

    def k_copy(t):
        return pltpu.make_async_copy(k_hbm.at[t], kbuf.at[t % NB], sem.at[SEM_K + t % NB])

    def v_copy(t):
        return pltpu.make_async_copy(v_hbm.at[t], vbuf.at[t % NB], sem.at[SEM_V + t % NB])

    def wq_copy(h):
        return pltpu.make_async_copy(wq_hbm.at[:, pl.ds(h * W, W)], wq_v.at[h], sem.at[SEM_WQ + h])

    def wo_copy(h):
        return pltpu.make_async_copy(wot_hbm.at[:, pl.ds(h * W, W)], wo_v.at[h], sem.at[SEM_WO + h])

    x_copy = pltpu.make_async_copy(x_hbm, x_v, sem.at[SEM_X])

    def o_copy(b):
        return pltpu.make_async_copy(ostage.at[b % 2], out_hbm.at[b], sem.at[SEM_O + b % 2])

    def fold(a, op):
        r = a[:, 0:LANES]
        for c in range(1, a.shape[1] // LANES):
            r = op(r, a[:, c * LANES:(c + 1) * LANES])
        return r

    def qproj_all(h):
        x = x_v[...]
        for r in range(rep):
            q_r = jnp.dot(x, wq_v[h, :, r * Dh:(r + 1) * Dh], preferred_element_type=jnp.float32)
            q_r = (q_r.astype(jnp.bfloat16) * scale).astype(jnp.bfloat16)
            for b in range(B):
                q_all[b * Hkv + h, r * Sq:(r + 1) * Sq, :] = q_r[b * Sq:(b + 1) * Sq]

    def qk(t, q, j, mx):
        s = lax.dot_general(q, kbuf[t % NB, j * CH:(j + 1) * CH, :], NT,
                            preferred_element_type=jnp.float32)
        s_buf[:, j * CH:(j + 1) * CH] = s
        f = fold(s, jnp.maximum)
        return f if mx is None else jnp.maximum(mx, f)

    def a_fin(mx):
        m = jnp.max(mx, axis=-1, keepdims=True)
        m_buf[...] = jnp.broadcast_to(m, (R, LANES))

    def expc(j, ls):
        m = m_buf[...]
        m2 = jnp.concatenate([m] * (CH // LANES), axis=1)
        p = jnp.exp(s_buf[:, j * CH:(j + 1) * CH] - m2)
        f = fold(p, jnp.add)
        return p.astype(jnp.bfloat16), (f if ls is None else ls + f)

    def pv(t, j, p, o):
        d = jnp.dot(p, vbuf[t % NB, j * CH:(j + 1) * CH, :], preferred_element_type=jnp.float32)
        return d if o is None else o + d

    def b_fin(t, o, ls):
        h = t % Hkv
        l = jnp.sum(ls, axis=-1, keepdims=True)
        o = (o / l).astype(jnp.bfloat16)
        o_cat = jnp.concatenate([o[r * Sq:(r + 1) * Sq] for r in range(rep)], axis=1)
        acc[...] += lax.dot_general(o_cat, wo_v[h], NT, preferred_element_type=jnp.float32)

    def stage_a(t):
        q = q_all[t]
        mx = None
        for j in range(NC):
            mx = qk(t, q, j, mx)
        a_fin(mx)

    def stage_b(t):
        o = None
        p_next, ls = expc(0, None)
        for j in range(NC):
            p = p_next
            if j + 1 < NC:
                p_next, ls = expc(j + 1, ls)
            o = pv(t, j, p, o)
        b_fin(t, o, ls)

    def stage_ab(tb):
        ta = tb + 1
        o = None
        q = q_all[ta]
        p_next, ls = expc(0, None)
        mx = qk(ta, q, 0, None)
        nq = 1
        for j in range(NC):
            p = p_next
            if j + 1 < NC:
                p_next, ls = expc(j + 1, ls)
            o = pv(tb, j, p, o)
            if nq < NC - LAG:
                mx = qk(ta, q, nq, mx)
                nq += 1
        while nq < NC:
            mx = qk(ta, q, nq, mx)
            nq += 1
        a_fin(mx)
        b_fin(tb, o, ls)

    def stage_split1(tb):
        ta = tb + 1
        ls = None
        mx = None
        q = q_all[ta]
        for j in range(NC):
            p, ls = expc(j, ls)
            p_buf[:, j * CH:(j + 1) * CH] = p
            mx = qk(ta, q, j, mx)
        l_buf[...] = ls
        a_fin(mx)

    def stage_split2(tb):
        o = jnp.dot(p_buf[...], vbuf[tb % NB], preferred_element_type=jnp.float32)
        b_fin(tb, o, l_buf[...])

    def finish_batch(t):
        b = t // Hkv

        @pl.when(t % Hkv == Hkv - 1)
        def _():
            @pl.when(b >= 2)
            def _():
                o_copy(b - 2).wait()
            ostage[b % 2] = acc[...].astype(ostage.dtype)
            acc[...] = jnp.zeros_like(acc)
            o_copy(b).start()

    x_copy.start()
    for h in range(Hkv):
        wq_copy(h).start()
    k_copy(0).start()
    for t in range(1, max(NB, Hkv + 1)):
        if t < NB:
            k_copy(t).start()
        if t - 1 < Hkv:
            wo_copy(t - 1).start()
        if t < NB:
            v_copy(t - 1).start()
    acc[...] = jnp.zeros_like(acc)
    x_copy.wait()

    def qbody(h, carry):
        wq_copy(h).wait()
        qproj_all(h)
        return carry

    lax.fori_loop(0, Hkv, qbody, 0)

    k_copy(0).wait()
    stage_a(0)

    def issue(i):
        @pl.when(i + NB < T)
        def _():
            k_copy(i + NB).start()

        @pl.when(i + NB - 1 < T)
        def _():
            v_copy(i + NB - 1).start()

    def body(i, carry):
        issue(i)

        @pl.when(i < Hkv)
        def _():
            wo_copy(i).wait()
        k_copy(i + 1).wait()
        v_copy(i).wait()
        stage_ab(i)
        finish_batch(i)
        return carry

    def body_split(i, carry):
        issue(i)
        k_copy(i + 1).wait()
        stage_split1(i)
        v_copy(i).wait()
        stage_split2(i)
        finish_batch(i)
        return carry

    n_fused = T - 1 - NSPLIT
    assert n_fused >= Hkv
    lax.fori_loop(0, n_fused, body, 0)
    lax.fori_loop(n_fused, T - 1, body_split, 0)

    v_copy(T - 1).wait()
    stage_b(T - 1)
    finish_batch(T - 1)
    o_copy(B - 2).wait()
    o_copy(B - 1).wait()


@jax.jit
def pallas_standalone__gqa_block_cached__near_ridge_kernel(
    x: jax.Array,
    k_cache: jax.Array,
    v_cache: jax.Array,
    wq: jax.Array,
    wo: jax.Array,
):
    B, Sq, D = x.shape
    _, Hkv, Sk, Dh = k_cache.shape
    Hq = wq.shape[1] // Dh
    rep = Hq // Hkv
    scale = Dh ** -0.5
    W = rep * Dh
    k3 = k_cache.reshape(B * Hkv, Sk, Dh)
    v3 = v_cache.reshape(B * Hkv, Sk, Dh)
    x2 = x.reshape(B * Sq, D)
    wot = wo.T

    kernel = functools.partial(_kernel, B=B, Hkv=Hkv, rep=rep, Sq=Sq, Sk=Sk, Dh=Dh, scale=scale)
    any_spec = pl.BlockSpec(memory_space=pl.ANY)
    return pl.pallas_call(
        kernel,
        in_specs=[any_spec] * 5,
        out_specs=any_spec,
        out_shape=jax.ShapeDtypeStruct((B, Sq, D), x.dtype),
        scratch_shapes=[
            pltpu.VMEM((B * Sq, D), x.dtype),
            pltpu.VMEM((Hkv, D, W), wq.dtype),
            pltpu.VMEM((Hkv, D, W), wo.dtype),
            pltpu.VMEM((B * Hkv, rep * Sq, Dh), jnp.bfloat16),
            pltpu.VMEM((NB, Sk, Dh), k_cache.dtype),
            pltpu.VMEM((NB, Sk, Dh), v_cache.dtype),
            pltpu.VMEM((rep * Sq, Sk), jnp.float32),
            pltpu.VMEM((rep * Sq, LANES), jnp.float32),
            pltpu.VMEM((rep * Sq, Sk), jnp.bfloat16),
            pltpu.VMEM((rep * Sq, LANES), jnp.float32),
            pltpu.VMEM((Sq, D), jnp.float32),
            pltpu.VMEM((2, Sq, D), x.dtype),
            pltpu.SemaphoreType.DMA((1 + 2 * Hkv + 2 * NB + 2,)),
        ],
        compiler_params=pltpu.CompilerParams(vmem_limit_bytes=64 * 1024 * 1024),
    )(x2, k3, v3, wq, wot)
```

```python
import functools

import jax
import jax.numpy as jnp
from jax import lax
import jax.experimental.pallas as pl
import jax.experimental.pallas.tpu as pltpu

NBV = 8
CH = 256
LAG = 2
JS = 8
LANES = 128
HI, LO = 0, 1
SIZES = [64, 64] + [48] * 31 + [96, 96, 240]
HR = 768


def _kernel(x_hbm, k_hbm, v_hbm, wq_hbm, wot_hbm, out_hbm,
            x_v, wq_v, wo_v, q_all, kh0, kh1, kt0, kt1, vbuf, s_buf, m_buf, p_buf, l_buf, acc,
            ostage, sem, *, B, Hkv, rep, Sq, Sk, Dh, scale):
    T = B * Hkv
    W = rep * Dh
    NC = Sk // CH
    R = rep * Sq
    kh = (kh0, kh1)
    kt = (kt0, kt1)
    assert HR % CH == 0 and sum(SIZES) == Sk and len(SIZES) == 4 * NC + 4
    pieces = []
    r = HR
    for n in SIZES:
        if r == Sk:
            r = 0
        pieces.append((r, n, r < HR))
        r += n
        assert r <= Sk
    assert r == HR
    SEM_X = 0
    SEM_WQ = 1
    SEM_WO = SEM_WQ + Hkv
    SEM_K = SEM_WO + Hkv
    SEM_V = SEM_K + 2
    SEM_O = SEM_V + NBV
    NT = (((1,), (1,)), ((), ()))

    def k_rows(par, r0):
        return (kh[par], r0) if r0 < HR else (kt[par], r0 - HR)

    def k_piece(t, par, r0, n):
        ref, r = k_rows(par, r0)
        return pltpu.make_async_copy(k_hbm.at[t, pl.ds(r0, n)], ref.at[pl.ds(r, n)],
                                     sem.at[SEM_K + par])

    def k_start(t, par):
        k_piece(t, par, 0, HR).start(priority=LO)
        k_piece(t, par, HR, Sk - HR).start(priority=LO)

    def k_wait(t, par):
        k_piece(t, par, 0, HR).wait()
        k_piece(t, par, HR, Sk - HR).wait()

    def v_copy(t):
        return pltpu.make_async_copy(v_hbm.at[t], vbuf.at[t % NBV], sem.at[SEM_V + t % NBV])

    def wq_copy(h):
        return pltpu.make_async_copy(wq_hbm.at[:, pl.ds(h * W, W)], wq_v.at[h], sem.at[SEM_WQ + h])

    def wo_copy(h):
        return pltpu.make_async_copy(wot_hbm.at[:, pl.ds(h * W, W)], wo_v.at[h], sem.at[SEM_WO + h])

    x_copy = pltpu.make_async_copy(x_hbm, x_v, sem.at[SEM_X])

    def o_copy(b):
        return pltpu.make_async_copy(ostage.at[b % 2], out_hbm.at[b], sem.at[SEM_O + b % 2])

    def fold(a, op):
        r = a[:, 0:LANES]
        for c in range(1, a.shape[1] // LANES):
            r = op(r, a[:, c * LANES:(c + 1) * LANES])
        return r

    def qproj_all(h):
        x = x_v[...]
        for r in range(rep):
            q_r = jnp.dot(x, wq_v[h, :, r * Dh:(r + 1) * Dh], preferred_element_type=jnp.float32)
            q_r = (q_r.astype(jnp.bfloat16) * scale).astype(jnp.bfloat16)
            for b in range(B):
                q_all[b * Hkv + h, r * Sq:(r + 1) * Sq, :] = q_r[b * Sq:(b + 1) * Sq]

    class Trickle:
        def __init__(self, tb, parb, level):
            self.tb, self.parb, self.level, self.n = tb, parb, level, 0

        def __call__(self, tile):
            r0, n, second = pieces[self.n]
            self.n += 1
            if self.level < (2 if second else 1):
                return
            t, par = (self.tb + 3, 1 - self.parb) if second else (self.tb + 2, self.parb)
            if tile is not None:
                ref, r = k_rows(par, r0)
                ref[r:r + 16, 0:LANES] = tile.astype(ref.dtype)
            k_piece(t, par, r0, n).start(priority=HI)

        def done(self):
            assert self.n == len(pieces)

    def qk(par, q, j, mx, tr=None):
        ref, r = k_rows(par, j * CH)
        s = lax.dot_general(q, ref[r:r + CH, :], NT, preferred_element_type=jnp.float32)
        s_buf[:, j * CH:(j + 1) * CH] = s
        if tr is not None:
            tr(s[R // 2 - 16:R // 2, 0:LANES])
            tr(s[R - 16:R, CH - LANES:CH])
        f = fold(s, jnp.maximum)
        return f if mx is None else jnp.maximum(mx, f)

    def a_fin(mx):
        m = jnp.max(mx, axis=-1, keepdims=True)
        m_buf[...] = jnp.broadcast_to(m, (R, LANES))

    def expc(j, ls, tr=None):
        m = m_buf[...]
        m2 = jnp.concatenate([m] * (CH // LANES), axis=1)
        p = jnp.exp(s_buf[:, j * CH:(j + 1) * CH] - m2)
        f = fold(p, jnp.add)
        if tr is not None:
            tr(p[R - 16:R, CH - LANES:CH])
        return p.astype(jnp.bfloat16), (f if ls is None else ls + f)

    def pv(t, j, p, o, tr=None):
        d = jnp.dot(p, vbuf[t % NBV, j * CH:(j + 1) * CH, :], preferred_element_type=jnp.float32)
        o = d if o is None else o + d
        if tr is not None:
            tr(o[R // 2 - 16:R // 2, 0:LANES])
            tr(o[R - 16:R, Dh - LANES:Dh])
        return o

    def b_fin(t, o, ls, tr=None):
        h = t % Hkv
        l = jnp.sum(ls, axis=-1, keepdims=True)
        o = o / l
        if tr is not None:
            tr(o[R - 16:R, Dh - LANES:Dh])
        o = o.astype(jnp.bfloat16)
        o_cat = jnp.concatenate([o[r * Sq:(r + 1) * Sq] for r in range(rep)], axis=1)
        contrib = lax.dot_general(o_cat, wo_v[h], NT, preferred_element_type=jnp.float32)
        if tr is not None:
            tr(contrib[Sq - 16:Sq, 2 * LANES:3 * LANES])
        acc[...] += contrib

    def stage_a(t, par):
        q = q_all[t]
        mx = None
        for j in range(NC):
            mx = qk(par, q, j, mx)
        a_fin(mx)

    def stage_b(t):
        o = None
        p_next, ls = expc(0, None)
        for j in range(NC):
            p = p_next
            if j + 1 < NC:
                p_next, ls = expc(j + 1, ls)
            o = pv(t, j, p, o)
        b_fin(t, o, ls)

    def stage_ab(tb, parb, tr):
        ta = tb + 1
        para = 1 - parb
        o = None
        q = q_all[ta]
        tr(None)
        p_next, ls = expc(0, None, tr)
        mx = qk(para, q, 0, None, tr)
        nq = 1
        for j in range(NC):
            p = p_next
            if j + 1 < NC:
                p_next, ls = expc(j + 1, ls)
            o = pv(tb, j, p, o, tr)
            if nq < NC - LAG:
                mx = qk(para, q, nq, mx, tr)
                nq += 1
        while nq < NC:
            mx = qk(para, q, nq, mx, tr)
            nq += 1
        a_fin(mx)
        b_fin(tb, o, ls, tr)
        tr.done()

    def stage_split1(tb, parb, tr):
        ta = tb + 1
        para = 1 - parb
        ls = None
        mx = None
        q = q_all[ta]
        tr(None)
        for j in range(NC):
            p, ls = expc(j, ls, tr if j == 0 else None)
            p_buf[:, j * CH:(j + 1) * CH] = p
            mx = qk(para, q, j, mx, tr)
        l_buf[...] = ls
        a_fin(mx)

    def stage_split2(tb, tr):
        o = None
        for j in range(NC):
            o = pv(tb, j, p_buf[:, j * CH:(j + 1) * CH], o, tr)
        b_fin(tb, o, l_buf[...], tr)
        tr.done()

    def finish_batch(t):
        b = t // Hkv

        @pl.when(t % Hkv == Hkv - 1)
        def _():
            @pl.when(b >= 2)
            def _():
                o_copy(b - 2).wait()
            ostage[b % 2] = acc[...].astype(ostage.dtype)
            acc[...] = jnp.zeros_like(acc)
            o_copy(b).start(priority=LO)

    x_copy.start(priority=LO)
    for h in range(Hkv):
        wq_copy(h).start(priority=LO)
    k_start(0, 0)
    k_start(1, 1)
    for t in range(max(NBV - 1, Hkv)):
        if t < Hkv:
            wo_copy(t).start(priority=LO)
        if t < NBV - 1:
            v_copy(t).start(priority=LO)
    acc[...] = jnp.zeros_like(acc)
    x_copy.wait()

    def qbody(h, carry):
        wq_copy(h).wait()
        qproj_all(h)
        return carry

    lax.fori_loop(0, Hkv, qbody, 0)
    k_wait(0, 0)
    stage_a(0, 0)
    k_piece(2, 0, 0, HR).start(priority=HI)

    def issue_v(i):
        @pl.when(i + NBV - 1 < T)
        def _():
            v_copy(i + NBV - 1).start(priority=LO)

    def block(i, par, level):
        issue_v(i)

        @pl.when(i < Hkv)
        def _():
            wo_copy(i).wait()
        k_wait(i + 1, 1 - par)
        v_copy(i).wait()
        stage_ab(i, par, Trickle(i, par, level))

    def block_split(i, par, level):
        issue_v(i)
        tr = Trickle(i, par, level)
        k_wait(i + 1, 1 - par)
        stage_split1(i, par, tr)
        v_copy(i).wait()
        stage_split2(i, tr)

    def body(j, carry):
        block(2 * j, 0, 2)
        block(2 * j + 1, 1, 2)
        finish_batch(2 * j + 1)
        return carry

    def body_split(j, carry):
        block_split(2 * j, 0, 2)
        block_split(2 * j + 1, 1, 2)
        finish_batch(2 * j + 1)
        return carry

    n_fused = T // 2 - 2 - JS
    assert T % 2 == 0 and Hkv % 2 == 0 and 2 * n_fused >= Hkv
    lax.fori_loop(0, n_fused, body, 0)
    lax.fori_loop(n_fused, T // 2 - 2, body_split, 0)
    block_split(T - 4, 0, 2)
    block_split(T - 3, 1, 1)
    block_split(T - 2, 0, 0)

    v_copy(T - 1).wait()
    stage_b(T - 1)
    finish_batch(T - 1)
    o_copy(B - 2).wait()
    o_copy(B - 1).wait()


@jax.jit
def pallas_standalone__gqa_block_cached__near_ridge_kernel(
    x: jax.Array,
    k_cache: jax.Array,
    v_cache: jax.Array,
    wq: jax.Array,
    wo: jax.Array,
):
    B, Sq, D = x.shape
    _, Hkv, Sk, Dh = k_cache.shape
    Hq = wq.shape[1] // Dh
    rep = Hq // Hkv
    scale = Dh ** -0.5
    W = rep * Dh
    k3 = k_cache.reshape(B * Hkv, Sk, Dh)
    v3 = v_cache.reshape(B * Hkv, Sk, Dh)
    x2 = x.reshape(B * Sq, D)
    wot = wo.T

    kernel = functools.partial(_kernel, B=B, Hkv=Hkv, rep=rep, Sq=Sq, Sk=Sk, Dh=Dh, scale=scale)
    any_spec = pl.BlockSpec(memory_space=pl.ANY)
    return pl.pallas_call(
        kernel,
        in_specs=[any_spec] * 5,
        out_specs=any_spec,
        out_shape=jax.ShapeDtypeStruct((B, Sq, D), x.dtype),
        scratch_shapes=[
            pltpu.VMEM((B * Sq, D), x.dtype),
            pltpu.VMEM((Hkv, D, W), wq.dtype),
            pltpu.VMEM((Hkv, D, W), wo.dtype),
            pltpu.VMEM((B * Hkv, rep * Sq, Dh), jnp.bfloat16),
            pltpu.VMEM((HR, Dh), k_cache.dtype),
            pltpu.VMEM((HR, Dh), k_cache.dtype),
            pltpu.VMEM((Sk - HR, Dh), k_cache.dtype),
            pltpu.VMEM((Sk - HR, Dh), k_cache.dtype),
            pltpu.VMEM((NBV, Sk, Dh), v_cache.dtype),
            pltpu.VMEM((rep * Sq, Sk), jnp.float32),
            pltpu.VMEM((rep * Sq, LANES), jnp.float32),
            pltpu.VMEM((rep * Sq, Sk), jnp.bfloat16),
            pltpu.VMEM((rep * Sq, LANES), jnp.float32),
            pltpu.VMEM((Sq, D), jnp.float32),
            pltpu.VMEM((2, Sq, D), x.dtype),
            pltpu.SemaphoreType.DMA((1 + 2 * Hkv + 2 + NBV + 2,)),
        ],
        compiler_params=pltpu.CompilerParams(
            vmem_limit_bytes=64 * 1024 * 1024,
            disable_bounds_checks=True,
            disable_semaphore_checks=True,
        ),
    )(x2, k3, v3, wq, wot)
```

```python
import functools

import jax
import jax.numpy as jnp
from jax import lax
import jax.experimental.pallas as pl
import jax.experimental.pallas.tpu as pltpu

NBV = 8
CH = 256
LAG = 2
NSPLIT = 11
LANES = 128
SUB = 16
HI, LO = 0, 1
SIZES = [64, 64] + [48] * 31 + [96, 96, 240]
HR = 768
WO_ROWS = 32


def _kernel(x_hbm, k_hbm, v_hbm, wq_hbm, wot_hbm, out_hbm,
            x_v, wq_v, wo_v, q_all, kh0, kh1, kt0, kt1, vbuf, s_buf, m_buf, p_buf, l_buf, mx_buf,
            acc, ostage, sem, *, B, Hkv, rep, Sq, Sk, Dh, scale):
    T = B * Hkv
    W = rep * Dh
    D = x_v.shape[1]
    NC = Sk // CH
    R = rep * Sq
    kh = (kh0, kh1)
    kt = (kt0, kt1)
    assert HR % CH == 0 and sum(SIZES) == Sk and len(SIZES) == 4 * NC + 4
    assert Dh == 2 * LANES and D % WO_ROWS == 0 and D // WO_ROWS <= (W // LANES) * (B // 2)
    pieces = []
    r = HR
    for n in SIZES:
        if r == Sk:
            r = 0
        pieces.append((r, n, r < HR))
        r += n
        assert r <= Sk
    assert r == HR
    SEM_X = 0
    SEM_WQ = 1
    SEM_WO = SEM_WQ + Hkv
    SEM_K = SEM_WO + Hkv
    SEM_V = SEM_K + 2
    SEM_O = SEM_V + NBV
    NT = (((1,), (1,)), ((), ()))

    def k_rows(par, r0):
        return (kh[par], r0) if r0 < HR else (kt[par], r0 - HR)

    def k_piece(t, par, r0, n):
        ref, r = k_rows(par, r0)
        return pltpu.make_async_copy(k_hbm.at[t, pl.ds(r0, n)], ref.at[pl.ds(r, n)],
                                     sem.at[SEM_K + par])

    def k_start(t, par):
        k_piece(t, par, 0, HR).start(priority=LO)
        k_piece(t, par, HR, Sk - HR).start(priority=LO)

    def k_wait(t, par):
        k_piece(t, par, 0, HR).wait()
        k_piece(t, par, HR, Sk - HR).wait()

    def v_copy(t):
        return pltpu.make_async_copy(v_hbm.at[t], vbuf.at[t % NBV], sem.at[SEM_V + t % NBV])

    def wq_copy(h):
        return pltpu.make_async_copy(wq_hbm.at[:, pl.ds(h * W, W)], wq_v.at[h], sem.at[SEM_WQ + h])

    def wo_piece(h, r0, n):
        return pltpu.make_async_copy(wot_hbm.at[pl.ds(r0, n), pl.ds(h * W, W)],
                                     wo_v.at[h, pl.ds(r0, n)], sem.at[SEM_WO + h])

    x_copy = pltpu.make_async_copy(x_hbm, x_v, sem.at[SEM_X])

    def o_copy(b):
        return pltpu.make_async_copy(ostage.at[b % 2], out_hbm.at[b], sem.at[SEM_O + b % 2])

    def fold(a, op):
        r = a[:, 0:LANES]
        for c in range(1, a.shape[1] // LANES):
            r = op(r, a[:, c * LANES:(c + 1) * LANES])
        return r

    def qproj_all(h):
        x = x_v[...]
        a = 0
        for c in range(W // LANES):
            r, c0 = divmod(c * LANES, Dh)
            q_c = jnp.dot(x, wq_v[h, :, c * LANES:(c + 1) * LANES],
                          preferred_element_type=jnp.float32)
            q_c = (q_c.astype(jnp.bfloat16) * scale).astype(jnp.bfloat16)
            for b in range(B):
                q_all[b * Hkv + h, r * Sq:(r + 1) * Sq, c0:c0 + LANES] = q_c[b * Sq:(b + 1) * Sq]
                if b % 2 == 1 and a * WO_ROWS < D:
                    r0 = a * WO_ROWS
                    wo_v[h, r0:r0 + SUB, 0:LANES] = q_c[(b + 1) * Sq - SUB:(b + 1) * Sq]
                    wo_piece(h, r0, WO_ROWS).start(priority=HI)
                    a += 1

    class Trickle:
        def __init__(self, tb, parb, guard):
            self.tb, self.parb, self.guard, self.n = tb, parb, guard, 0

        def __call__(self, tile):
            r0, n, second = pieces[self.n]
            self.n += 1
            t, par = (self.tb + 3, 1 - self.parb) if second else (self.tb + 2, self.parb)
            if tile is not None:
                ref, r = k_rows(par, r0)
                ref[r:r + SUB, 0:LANES] = tile.astype(ref.dtype)
            if self.guard:
                @pl.when(t < T)
                def _():
                    k_piece(t, par, r0, n).start(priority=HI)
            else:
                k_piece(t, par, r0, n).start(priority=HI)

        def done(self):
            assert self.n == len(pieces)

    def qk(par, q, j, mx, tr=None):
        ref, r = k_rows(par, j * CH)
        s = lax.dot_general(q, ref[r:r + CH, :], NT, preferred_element_type=jnp.float32)
        s_buf[:, j * CH:(j + 1) * CH] = s
        if tr is not None:
            tr(s[R // 2 - SUB:R // 2, 0:LANES])
            tr(s[R - SUB:R, CH - LANES:CH])
        f = fold(s, jnp.maximum)
        return f if mx is None else jnp.maximum(mx, f)

    def a_fin(mx):
        m = jnp.max(mx, axis=-1, keepdims=True)
        m_buf[...] = jnp.broadcast_to(m, (R, LANES))

    def expc(j, ls, tr=None):
        m = m_buf[...]
        m2 = jnp.concatenate([m] * (CH // LANES), axis=1)
        p = jnp.exp(s_buf[:, j * CH:(j + 1) * CH] - m2)
        f = fold(p, jnp.add)
        if tr is not None:
            tr(p[R - SUB:R, CH - LANES:CH])
        return p.astype(jnp.bfloat16), (f if ls is None else ls + f)

    def pv(t, j, p, o, tr=None):
        d = jnp.dot(p, vbuf[t % NBV, j * CH:(j + 1) * CH, :], preferred_element_type=jnp.float32)
        o = d if o is None else o + d
        if tr is not None:
            tr(o[R // 2 - SUB:R // 2, 0:LANES])
            tr(o[R - SUB:R, Dh - LANES:Dh])
        return o

    def b_fin(t, o, ls, tr=None):
        h = t % Hkv
        l = jnp.sum(ls, axis=-1, keepdims=True)
        o = o / l
        if tr is not None:
            tr(o[R - SUB:R, Dh - LANES:Dh])
        o = o.astype(jnp.bfloat16)
        o_cat = jnp.concatenate([o[r * Sq:(r + 1) * Sq] for r in range(rep)], axis=1)
        contrib = lax.dot_general(o_cat, wo_v[h], NT, preferred_element_type=jnp.float32)
        if tr is not None:
            tr(contrib[Sq - SUB:Sq, 2 * LANES:3 * LANES])
        acc[...] += contrib

    def stage_a(t, par):
        q = q_all[t]
        mx = None
        for j in range(NC):
            mx = qk(par, q, j, mx)
        a_fin(mx)

    def stage_b(t):
        o = None
        p_next, ls = expc(0, None)
        for j in range(NC):
            p = p_next
            if j + 1 < NC:
                p_next, ls = expc(j + 1, ls)
            o = pv(t, j, p, o)
        b_fin(t, o, ls)

    def stage_ab(tb, parb, tr):
        ta = tb + 1
        para = 1 - parb
        o = None
        q = q_all[ta]
        tr(None)
        p_next, ls = expc(0, None, tr)
        mx = qk(para, q, 0, None, tr)
        nq = 1
        for j in range(NC):
            p = p_next
            if j + 1 < NC:
                p_next, ls = expc(j + 1, ls)
            o = pv(tb, j, p, o, tr)
            if nq < NC - LAG:
                mx = qk(para, q, nq, mx, tr)
                nq += 1
        while nq < NC:
            mx = qk(para, q, nq, mx, tr)
            nq += 1
        a_fin(mx)
        b_fin(tb, o, ls, tr)
        tr.done()

    def stage_split1(tb, parb, tr):
        ta = tb + 1
        para = 1 - parb
        ls = None
        mx = None
        q = q_all[ta]
        tr(None)
        for j in range(NC):
            p, ls = expc(j, ls, tr if j == 0 else None)
            p_buf[:, j * CH:(j + 1) * CH] = p
            mx = qk(para, q, j, mx, tr)
        l_buf[...] = ls
        mx_buf[...] = mx

    def stage_split2(tb, tr):
        a_fin(mx_buf[...])
        h = tb % Hkv
        l = jnp.sum(l_buf[...], axis=-1, keepdims=True)
        os_ = []
        for n in range(Dh // LANES):
            o = None
            for j in range(NC):
                d = jnp.dot(p_buf[:, j * CH:(j + 1) * CH],
                            vbuf[tb % NBV, j * CH:(j + 1) * CH, n * LANES:(n + 1) * LANES],
                            preferred_element_type=jnp.float32)
                o = d if o is None else o + d
                tr(o[R - SUB:R, :])
            os_.append(o)
        contrib = None
        for n in range(Dh // LANES):
            o = os_[n] / l
            if n == Dh // LANES - 1:
                tr(o[R - SUB:R, :])
            o = o.astype(jnp.bfloat16)
            for r in range(rep):
                c0 = r * Dh + n * LANES
                d = lax.dot_general(o[r * Sq:(r + 1) * Sq], wo_v[h, :, c0:c0 + LANES], NT,
                                    preferred_element_type=jnp.float32)
                contrib = d if contrib is None else contrib + d
        tr(contrib[Sq - SUB:Sq, 2 * LANES:3 * LANES])
        acc[...] += contrib
        tr.done()

    def finish_batch(t):
        b = t // Hkv

        @pl.when(t % Hkv == Hkv - 1)
        def _():
            @pl.when(b >= 2)
            def _():
                o_copy(b - 2).wait()
            ostage[b % 2] = acc[...].astype(ostage.dtype)
            acc[...] = jnp.zeros_like(acc)
            o_copy(b).start(priority=LO)

    x_copy.start(priority=LO)
    for h in range(Hkv):
        wq_copy(h).start(priority=LO)
    k_start(0, 0)
    k_start(1, 1)
    for t in range(NBV - 1):
        v_copy(t).start(priority=LO)
    acc[...] = jnp.zeros_like(acc)
    x_copy.wait()

    def qbody(h, carry):
        wq_copy(h).wait()
        qproj_all(h)
        return carry

    lax.fori_loop(0, Hkv, qbody, 0)
    k_wait(0, 0)
    stage_a(0, 0)
    k_piece(2, 0, 0, HR).start(priority=HI)

    def issue_v(i):
        @pl.when(i + NBV - 1 < T)
        def _():
            v_copy(i + NBV - 1).start(priority=LO)

    def block(i, par):
        issue_v(i)

        @pl.when(i < Hkv)
        def _():
            wo_piece(i, 0, D).wait()
        k_wait(i + 1, 1 - par)
        v_copy(i).wait()
        stage_ab(i, par, Trickle(i, par, False))

    def block_split(i, par):
        issue_v(i)
        tr = Trickle(i, par, True)
        k_wait(i + 1, 1 - par)
        stage_split1(i, par, tr)
        v_copy(i).wait()
        stage_split2(i, tr)

    def by_parity(fn):
        def body(i, carry):
            @pl.when(i % 2 == 0)
            def _():
                fn(i, 0)

            @pl.when(i % 2 == 1)
            def _():
                fn(i, 1)
                finish_batch(i)
            return carry
        return body

    n_fused = T - 1 - NSPLIT
    assert Hkv % 2 == 0 and Hkv <= n_fused <= T - 3 and NBV <= T
    lax.fori_loop(0, n_fused, by_parity(block), 0)
    lax.fori_loop(n_fused, T - 1, by_parity(block_split), 0)

    v_copy(T - 1).wait()
    stage_b(T - 1)
    finish_batch(T - 1)
    o_copy(B - 2).wait()
    o_copy(B - 1).wait()


@jax.jit
def pallas_standalone__gqa_block_cached__near_ridge_kernel(
    x: jax.Array,
    k_cache: jax.Array,
    v_cache: jax.Array,
    wq: jax.Array,
    wo: jax.Array,
):
    B, Sq, D = x.shape
    _, Hkv, Sk, Dh = k_cache.shape
    Hq = wq.shape[1] // Dh
    rep = Hq // Hkv
    scale = Dh ** -0.5
    W = rep * Dh
    k3 = k_cache.reshape(B * Hkv, Sk, Dh)
    v3 = v_cache.reshape(B * Hkv, Sk, Dh)
    x2 = x.reshape(B * Sq, D)
    wot = wo.T

    kernel = functools.partial(_kernel, B=B, Hkv=Hkv, rep=rep, Sq=Sq, Sk=Sk, Dh=Dh, scale=scale)
    any_spec = pl.BlockSpec(memory_space=pl.ANY)
    return pl.pallas_call(
        kernel,
        in_specs=[any_spec] * 5,
        out_specs=any_spec,
        out_shape=jax.ShapeDtypeStruct((B, Sq, D), x.dtype),
        scratch_shapes=[
            pltpu.VMEM((B * Sq, D), x.dtype),
            pltpu.VMEM((Hkv, D, W), wq.dtype),
            pltpu.VMEM((Hkv, D, W), wo.dtype),
            pltpu.VMEM((B * Hkv, rep * Sq, Dh), jnp.bfloat16),
            pltpu.VMEM((HR, Dh), k_cache.dtype),
            pltpu.VMEM((HR, Dh), k_cache.dtype),
            pltpu.VMEM((Sk - HR, Dh), k_cache.dtype),
            pltpu.VMEM((Sk - HR, Dh), k_cache.dtype),
            pltpu.VMEM((NBV, Sk, Dh), v_cache.dtype),
            pltpu.VMEM((rep * Sq, Sk), jnp.float32),
            pltpu.VMEM((rep * Sq, LANES), jnp.float32),
            pltpu.VMEM((rep * Sq, Sk), jnp.bfloat16),
            pltpu.VMEM((rep * Sq, LANES), jnp.float32),
            pltpu.VMEM((rep * Sq, LANES), jnp.float32),
            pltpu.VMEM((Sq, D), jnp.float32),
            pltpu.VMEM((2, Sq, D), x.dtype),
            pltpu.SemaphoreType.DMA((1 + 2 * Hkv + 2 + NBV + 2,)),
        ],
        compiler_params=pltpu.CompilerParams(
            vmem_limit_bytes=64 * 1024 * 1024,
            disable_bounds_checks=True,
            disable_semaphore_checks=True,
        ),
    )(x2, k3, v3, wq, wot)
```
